```python
import os as _os
_os.environ.setdefault("JAX_PLATFORMS", "cpu")
import jax
import jax.numpy as jnp

def _softmax(x, axis=-1):
    return jax.nn.softmax(x, axis=axis)
def _gelu(x):
    return jax.nn.gelu(x, approximate=True)
def _silu(x):
    return jax.nn.silu(x)
def _sigmoid(x):
    return jax.nn.sigmoid(x)
def _layernorm(x, axis=-1, eps=1e-5):
    m = jnp.mean(x, axis=axis, keepdims=True)
    v = jnp.var(x, axis=axis, keepdims=True)
    return (x - m) / jnp.sqrt(v + eps)
def _scatter_add(tgt, idx, src, axis=0):
    return tgt.at[idx].add(src)
def _segment_sum(src, seg, n):
    return jax.ops.segment_sum(src, seg, n)
class _Rng:
    def __init__(self, key):
        self._k = key
    def _next(self):
        self._k, sub = jax.random.split(self._k)
        return sub
    def normal(self, shape):
        return jax.random.normal(self._next(), shape, dtype=jnp.bfloat16)
    def randint(self, lo, hi, shape):
        return jax.random.randint(self._next(), shape, lo, hi, dtype=jnp.int32)
    def uniform(self, shape, lo=0.0, hi=1.0):
        return jax.random.uniform(self._next(), shape, jnp.bfloat16, lo, hi)
    def permutation(self, n):
        return jax.random.permutation(self._next(), n)


kernel_name = 'gated_mix__mha_block__softmax_full_mha__prompt'

def setup_inputs():
    _rng = _Rng(jax.random.key(int.from_bytes(__import__("os").urandom(4), "little")))
    _w = (lambda a: (lambda t: t.astype(jnp.bfloat16) if jnp.issubdtype(t.dtype, jnp.floating) else t)(jnp.asarray(a)))
    def _A_setup():
        B, S, D, H = 1, 2048, 448, 16
        return {
            "x": _w((lambda *s: _rng.normal(s) * 0.05)(B, S, D)),
            "wqkv": _w((lambda *s: _rng.normal(s) * 0.4)(D, 3 * D)),
            "wo": _w((lambda *s: _rng.normal(s) * 0.05)(D, D)),
        }
    _A_in = _A_setup()

    def _B_setup():
        B, S, D = 1, 2048, 448
        return {
            "x": _w((lambda *s: _rng.normal(s) * 0.05)(B, S, D)),
            "wqkv": _w((lambda *s: _rng.normal(s) * 0.4)(D, 3 * D)),
            "wo": _w((lambda *s: _rng.normal(s) * 0.05)(D, D)),
        }
    _B_in = _B_setup()

    return {
        "A_x": _A_in["x"],
        "A_wqkv": _A_in["wqkv"],
        "A_wo": _A_in["wo"],
        "B_x": _B_in["x"],
        "B_wqkv": _B_in["wqkv"],
        "B_wo": _B_in["wo"],
        "gate_w": _w((lambda *s: _rng.normal(s) * 0.05)(448) * 16.0),
    }

def reference(A_x, A_wqkv, A_wo, B_x, B_wqkv, B_wo, gate_w):
    def _A_ref(x, wqkv, wo):
        B, S, D = x.shape
        H = 16
        Dh = D // H
        qkv = (lambda x, *d: x.transpose(*d))((x @ wqkv).reshape(B, S, 3, H, Dh), 2, 0, 3, 1, 4)
        q, k, v = qkv[0], qkv[1], qkv[2]
        scores = jnp.einsum("bhqd,bhkd->bhqk", q, k) * (Dh ** -0.5)
        p = _softmax(scores, axis=-1)
        o = jnp.einsum("bhqk,bhkd->bhqd", p, v)
        return (lambda x, *d: x.transpose(*d))(o, 0, 2, 1, 3).reshape(B, S, D) @ wo

    def _B_ref(x, wqkv, wo):
        B, S, D = x.shape
        H = 16; Dh = D // H
        qkv = (lambda x, *d: x.transpose(*d))((x @ wqkv).reshape(B, S, 3, H, Dh), 2, 0, 3, 1, 4)
        q, k, v = qkv[0], qkv[1], qkv[2]
        scale = Dh ** -0.5
        scores = jnp.einsum("bhqd,bhkd->bhqk", q, k) * scale
        p = _softmax(scores, axis=-1)
        o = jnp.einsum("bhqk,bhkd->bhqd", p, v)
        return (lambda x, *d: x.transpose(*d))(o, 0, 2, 1, 3).reshape(B, S, D) @ wo

    x = A_x
    g = _sigmoid((x * gate_w).sum(-1, keepdims=True))
    a = _A_ref(x, A_wqkv, A_wo)
    b = _B_ref(x, B_wqkv, B_wo)
    return g * a + (1 - g) * b
```

```python
import functools, math
import jax, jax.numpy as jnp
from jax.experimental import pallas as pl
from jax.experimental.pallas import tpu as pltpu

S, D, H, DH = 2048, 448, 16, 28
DP = 32
NH = 2 * H
G = NH * DP // 128
LOG2E = 1.4426950408889634
F32, BF16 = jnp.float32, jnp.bfloat16

def make_kernel(TQ=512, KC=128):
    NC = S // KC
    def kernel(xt_ref, wa_ref, wb_ref, woa_ref, wob_ref, gw_ref, o_ref,
               k_scr, vt_scr, wqt_scr, wot_scr, tmp_scr, pad_scr, q_scr, sa_scr, sb_scr, ot_scr):
        i = pl.program_id(0)

        @pl.when(i == 0)
        def _():
            xt = xt_ref[...]
            x = xt.T
            for b, (w_ref, wo_ref) in enumerate(((wa_ref, woa_ref), (wb_ref, wob_ref))):
                tmp_scr[...] = w_ref[...].T.astype(F32)
                pad_scr[...] = jnp.zeros(pad_scr.shape, F32)
                for j in range(3 * H):
                    pad_scr[j * DP:j * DP + DH, :] = tmp_scr[j * DH:(j + 1) * DH, :]
                HP = H * DP
                wqt_scr[b * HP:(b + 1) * HP, :] = pad_scr[0:HP, :].astype(BF16)
                wk = pad_scr[HP:2 * HP, :].astype(BF16).T
                k = jnp.dot(x, wk, preferred_element_type=F32)
                for g in range(G // 2):
                    k_scr[b * (G // 2) + g] = k[:, g * 128:(g + 1) * 128].astype(BF16)
                vt = jnp.dot(pad_scr[2 * HP:3 * HP, :].astype(BF16), xt, preferred_element_type=F32)
                row = jax.lax.broadcasted_iota(jnp.int32, vt.shape, 0)
                vt = jnp.where(row % DP == DH, 1.0, vt)
                vt_scr[b * H:(b + 1) * H] = vt.astype(BF16).reshape(H, DP, S)
                tmp_scr[0:D, :] = wo_ref[...].astype(F32)
                pad_scr[0:HP, :] = jnp.zeros((HP, D), F32)
                for j in range(H):
                    pad_scr[j * DP:j * DP + DH, :] = tmp_scr[j * DH:(j + 1) * DH, :]
                wot_scr[:, b * HP:(b + 1) * HP] = pad_scr[0:HP, :].astype(BF16).T

        xq = xt_ref[:, pl.ds(pl.multiple_of(i * TQ, TQ), TQ)]
        qt = jnp.dot(wqt_scr[...], xq, preferred_element_type=F32) * (DH ** -0.5 * LOG2E)
        q_scr[...] = qt.astype(BF16).reshape(G, 128, TQ)
        gl = jnp.dot(jnp.broadcast_to(gw_ref[...], (8, D)), xq, preferred_element_type=F32)
        gate = jax.nn.sigmoid(gl[0:1, :])

        rowg = jax.lax.broadcasted_iota(jnp.int32, (128, TQ), 0) // DP

        def stage(h1, s1_ref, h2, s2_ref, m2):
            if h1 is not None:
                g = h1 // 4
                qg = q_scr[g]
                qm = jnp.where(rowg == (h1 % 4), qg, jnp.zeros_like(qg))
                mx = jnp.full((8, TQ), -jnp.inf, F32)
            if h2 is not None:
                acc = jnp.zeros((DP, TQ), F32)
            for c in range(NC):
                if h1 is not None:
                    s = jnp.dot(k_scr[g, c * KC:(c + 1) * KC, :], qm, preferred_element_type=F32)
                    s1_ref[c * KC:(c + 1) * KC, :] = s
                    mx = jnp.maximum(mx, s.reshape(KC // 8, 8, TQ).max(axis=0))
                if h2 is not None:
                    p = jnp.exp2(s2_ref[c * KC:(c + 1) * KC, :] - m2).astype(BF16)
                    acc = acc + jnp.dot(vt_scr[h2, :, c * KC:(c + 1) * KC], p, preferred_element_type=F32)
            if h2 is not None:
                l = acc[DH:DH + 1, :]
                gsel = jnp.where(h2 < H, gate, 1.0 - gate)
                ot_scr[h2] = (acc * (gsel / l)).astype(BF16)
            if h1 is not None:
                return mx.max(axis=0, keepdims=True)
            return None

        m0 = stage(0, sa_scr, None, None, None)

        def body(j, m):
            h = 2 * j
            mb = stage(h + 1, sb_scr, h, sa_scr, m)
            ma = stage(h + 2, sa_scr, h + 1, sb_scr, mb)
            return ma

        m = jax.lax.fori_loop(0, NH // 2 - 1, body, m0)
        mb = stage(NH - 1, sb_scr, NH - 2, sa_scr, m)
        stage(None, None, NH - 1, sb_scr, mb)

        ot = ot_scr[...].reshape(NH * DP, TQ)
        out = jnp.dot(wot_scr[...], ot, preferred_element_type=F32)
        o_ref[...] = out.astype(o_ref.dtype)

    def fn(A_x, A_wqkv, A_wo, B_x, B_wqkv, B_wo, gate_w):
        xt = jnp.transpose(A_x, (0, 2, 1)).reshape(D, S)
        gw = gate_w.reshape(1, D)
        full = lambda shp: pl.BlockSpec(shp, lambda i: (0,) * len(shp))
        out = pl.pallas_call(
            kernel,
            grid=(S // TQ,),
            in_specs=[full((D, S)), full((D, 3 * D)), full((D, 3 * D)), full((D, D)), full((D, D)), full((1, D))],
            out_specs=pl.BlockSpec((D, TQ), lambda i: (0, i)),
            out_shape=jax.ShapeDtypeStruct((D, S), BF16),
            scratch_shapes=[pltpu.VMEM((G, S, 128), BF16),
                            pltpu.VMEM((NH, DP, S), BF16),
                            pltpu.VMEM((NH * DP, D), BF16),
                            pltpu.VMEM((D, NH * DP), BF16),
                            pltpu.VMEM((3 * D, D), F32),
                            pltpu.VMEM((3 * H * DP, D), F32),
                            pltpu.VMEM((G, 128, TQ), BF16),
                            pltpu.VMEM((S, TQ), F32),
                            pltpu.VMEM((S, TQ), F32),
                            pltpu.VMEM((NH, DP, TQ), BF16)],
            compiler_params=pltpu.CompilerParams(dimension_semantics=("arbitrary",), vmem_limit_bytes=100 * 2**20),
        )(xt, A_wqkv, B_wqkv, A_wo, B_wo, gw)
        return jnp.transpose(out.reshape(1, D, S), (0, 2, 1))
    return fn


_impl = make_kernel(512, 128)


@jax.jit
def pallas_gated_mix__mha_block__softmax_full_mha__prompt_kernel(
    A_x: jax.Array,
    A_wqkv: jax.Array,
    A_wo: jax.Array,
    B_x: jax.Array,
    B_wqkv: jax.Array,
    B_wo: jax.Array,
    gate_w: jax.Array,
):
    return _impl(A_x, A_wqkv, A_wo, B_x, B_wqkv, B_wo, gate_w)
```

```python
import functools, math
import jax, jax.numpy as jnp
from jax.experimental import pallas as pl
from jax.experimental.pallas import tpu as pltpu

S, D, H, DH = 2048, 448, 16, 28
DP = 32
HP = H * DP
NH = 2 * H
G = NH * DP // 128
LOG2E = 1.4426950408889634
F32, BF16 = jnp.float32, jnp.bfloat16

def make_kernel(TQ=512, KC=128, U=4, XC=4):
    NC = S // KC
    XW = S // XC
    def kernel(xt_hbm, wa_hbm, wb_hbm, woa_hbm, wob_hbm, gw_ref, o_ref,
               xt_v, w_v, wo_v, sems,
               k_scr, vt_scr, wqt_scr, wot_scr, tmp_scr, pad_scr, tmpo_scr, pado_scr, wk_scr, wvt_scr, x_scr, q_scr, sa_scr, sb_scr, ot_scr, po_scr):
        i = pl.program_id(0)

        @pl.when(i == 0)
        def _():
            cp_w = [pltpu.make_async_copy(src, w_v.at[b], sems.at[b]) for b, src in enumerate((wa_hbm, wb_hbm))]
            cp_wo = [pltpu.make_async_copy(src, wo_v.at[b], sems.at[2 + b]) for b, src in enumerate((woa_hbm, wob_hbm))]
            cp_x = [pltpu.make_async_copy(xt_hbm.at[:, c * XW:(c + 1) * XW], xt_v.at[:, c * XW:(c + 1) * XW],
                                          sems.at[4 + c]) for c in range(XC)]
            cp_w[0].start()
            for c in range(XC):
                cp_x[c].start()
            cp_w[1].start()
            cp_wo[0].start()
            cp_wo[1].start()

            def prep_qkv(b):
                tmp_scr[b] = w_v[b].T.astype(F32)
                for part in (2, 1, 0):
                    for j in range(part * H, (part + 1) * H):
                        pad_scr[b, j * DP:j * DP + DH, :] = tmp_scr[b, j * DH:(j + 1) * DH, :]
                        pad_scr[b, j * DP + DH:(j + 1) * DP, :] = jnp.zeros((DP - DH, D), F32)
                    w = pad_scr[b, part * HP:(part + 1) * HP, :].astype(BF16)
                    if part == 2:
                        wvt_scr[b] = w
                    elif part == 1:
                        wk_scr[b] = w.T
                    else:
                        wqt_scr[b * HP:(b + 1) * HP, :] = w

            def prep_wo(b):
                tmpo_scr[b] = wo_v[b].astype(F32)
                for j in range(H):
                    pado_scr[b, j * DP:j * DP + DH, :] = tmpo_scr[b, j * DH:(j + 1) * DH, :]
                    pado_scr[b, j * DP + DH:(j + 1) * DP, :] = jnp.zeros((DP - DH, D), F32)
                wot_scr[:, b * HP:(b + 1) * HP] = pado_scr[b].astype(BF16).T

            def kv_chunk(b, c):
                vt = jnp.dot(wvt_scr[b], xt_v[:, c * XW:(c + 1) * XW], preferred_element_type=F32)
                row = jax.lax.broadcasted_iota(jnp.int32, vt.shape, 0)
                vt = jnp.where(row % DP == DH, 1.0, vt)
                vt_scr[b * H:(b + 1) * H, :, c * XW:(c + 1) * XW] = vt.astype(BF16).reshape(H, DP, XW)
                k = jnp.dot(x_scr[c * XW:(c + 1) * XW, :], wk_scr[b], preferred_element_type=F32)
                for g in range(G // 2):
                    k_scr[b * (G // 2) + g, c * XW:(c + 1) * XW, :] = k[:, g * 128:(g + 1) * 128].astype(BF16)

            cp_w[0].wait()
            cp_x[0].wait()
            prep_qkv(0)
            x_scr[0:XW, :] = xt_v[:, 0:XW].T
            kv_chunk(0, 0)
            for c in range(1, XC):
                cp_x[c].wait()
            cp_w[1].wait()
            cp_wo[0].wait()
            cp_wo[1].wait()
            for c in range(1, XC):
                x_scr[c * XW:(c + 1) * XW, :] = xt_v[:, c * XW:(c + 1) * XW].T
                if c == 1:
                    prep_qkv(1)
                if c == min(2, XC - 1):
                    prep_wo(0)
                    prep_wo(1)
                kv_chunk(0, c)
            for c in range(XC):
                kv_chunk(1, c)

        xq = xt_v[:, pl.ds(pl.multiple_of(i * TQ, TQ), TQ)]
        qt = jnp.dot(wqt_scr[...], xq, preferred_element_type=F32) * (DH ** -0.5 * LOG2E)
        q_scr[...] = qt.astype(BF16).reshape(G, 128, TQ)
        gl = jnp.dot(jnp.broadcast_to(gw_ref[...], (8, D)), xq, preferred_element_type=F32)
        gate = jax.nn.sigmoid(gl[0:1, :])

        rowg = jax.lax.broadcasted_iota(jnp.int32, (128, TQ), 0) // DP

        def stage(h1, s1_ref, h2, s2_ref, m2, extra=None):
            if h1 is not None:
                g = h1 // 4
                qg = q_scr[g]
                qm = jnp.where(rowg == (h1 % 4), qg, jnp.zeros_like(qg))
                mx = jnp.full((8, TQ), -jnp.inf, F32)
            if h2 is not None:
                acc = jnp.zeros((DP, TQ), F32)
            for c in range(NC):
                if h1 is not None:
                    s = jnp.dot(k_scr[g, c * KC:(c + 1) * KC, :], qm, preferred_element_type=F32)
                    s1_ref[c * KC:(c + 1) * KC, :] = s
                    mx = jnp.maximum(mx, s.reshape(KC // 8, 8, TQ).max(axis=0))
                if h2 is not None:
                    p = jnp.exp2(s2_ref[c * KC:(c + 1) * KC, :] - m2).astype(BF16)
                    acc = acc + jnp.dot(vt_scr[h2, :, c * KC:(c + 1) * KC], p, preferred_element_type=F32)
                if extra is not None:
                    extra(c)
            if h2 is not None:
                l = acc[DH:DH + 1, :]
                gsel = jnp.where(h2 < H, gate, 1.0 - gate)
                ot_scr[h2] = (acc * (gsel / l)).astype(BF16)
            if h1 is not None:
                return mx.max(axis=0, keepdims=True)
            return None

        bufs = (sa_scr, sb_scr)
        m = stage(0, sa_scr, None, None, None)
        NIT = (NH - 1) // U

        def body(j, m):
            for u in range(U):
                k = j * U + 1 + u
                m = stage(k, bufs[(1 + u) % 2], k - 1, bufs[u % 2], m)
            return m

        if NIT > 0:
            m = jax.lax.fori_loop(0, NIT, body, m)
        for k in range(NIT * U + 1, NH):
            m = stage(k, bufs[k % 2], k - 1, bufs[(k - 1) % 2], m)
        KS = (NH - 4) * DP
        RB = 64
        def extra(c):
            if c % 2 == 0 and c // 2 < D // RB:
                r = c // 2
                po_scr[r * RB:(r + 1) * RB, :] = jnp.dot(wot_scr[r * RB:(r + 1) * RB, :KS], ot_scr[:NH - 4].reshape(KS, TQ),
                                                         preferred_element_type=F32)
        stage(None, None, NH - 1, bufs[(NH - 1) % 2], m, extra)
        out = po_scr[...] + jnp.dot(wot_scr[:, KS:], ot_scr[NH - 4:].reshape(4 * DP, TQ), preferred_element_type=F32)
        o_ref[...] = out.astype(o_ref.dtype)

    def fn(A_x, A_wqkv, A_wo, B_x, B_wqkv, B_wo, gate_w):
        xt = jnp.transpose(A_x, (0, 2, 1)).reshape(D, S)
        gw = gate_w.reshape(1, D)
        anyspec = pl.BlockSpec(memory_space=pl.ANY)
        out = pl.pallas_call(
            kernel,
            grid=(S // TQ,),
            in_specs=[anyspec, anyspec, anyspec, anyspec, anyspec, pl.BlockSpec((1, D), lambda i: (0, 0))],
            out_specs=pl.BlockSpec((D, TQ), lambda i: (0, i)),
            out_shape=jax.ShapeDtypeStruct((D, S), BF16),
            scratch_shapes=[pltpu.VMEM((D, S), BF16),
                            pltpu.VMEM((2, D, 3 * D), BF16),
                            pltpu.VMEM((2, D, D), BF16),
                            pltpu.SemaphoreType.DMA((4 + XC,)),
                            pltpu.VMEM((G, S, 128), BF16),
                            pltpu.VMEM((NH, DP, S), BF16),
                            pltpu.VMEM((NH * DP, D), BF16),
                            pltpu.VMEM((D, NH * DP), BF16),
                            pltpu.VMEM((2, 3 * D, D), F32),
                            pltpu.VMEM((2, 3 * HP, D), F32),
                            pltpu.VMEM((2, D, D), F32),
                            pltpu.VMEM((2, HP, D), F32),
                            pltpu.VMEM((2, D, HP), BF16),
                            pltpu.VMEM((2, HP, D), BF16),
                            pltpu.VMEM((S, D), BF16),
                            pltpu.VMEM((G, 128, TQ), BF16),
                            pltpu.VMEM((S, TQ), F32),
                            pltpu.VMEM((S, TQ), F32),
                            pltpu.VMEM((NH, DP, TQ), BF16),
                            pltpu.VMEM((D, TQ), F32)],
            compiler_params=pltpu.CompilerParams(dimension_semantics=("arbitrary",), vmem_limit_bytes=100 * 2**20),
        )(xt, A_wqkv, B_wqkv, A_wo, B_wo, gw)
        return jnp.transpose(out.reshape(1, D, S), (0, 2, 1))
    return fn


_impl = make_kernel(512, 128, 6, 2)


@jax.jit
def pallas_gated_mix__mha_block__softmax_full_mha__prompt_kernel(
    A_x: jax.Array,
    A_wqkv: jax.Array,
    A_wo: jax.Array,
    B_x: jax.Array,
    B_wqkv: jax.Array,
    B_wo: jax.Array,
    gate_w: jax.Array,
):
    return _impl(A_x, A_wqkv, A_wo, B_x, B_wqkv, B_wo, gate_w)
```

```python
import functools, math
import jax, jax.numpy as jnp
from jax.experimental import pallas as pl
from jax.experimental.pallas import tpu as pltpu

S, D, H, DH = 2048, 448, 16, 28
DP = 32
HP = H * DP
NH = 2 * H
G = NH * DP // 128
LOG2E = 1.4426950408889634
F32, BF16 = jnp.float32, jnp.bfloat16

def make_kernel(TQ=512, KC=128, U=4, XC=4, LAG=1):
    NC = S // KC
    XW = S // XC
    def kernel(xt_hbm, wa_hbm, wb_hbm, woa_hbm, wob_hbm, gw_ref, o_ref,
               xt_v, w_v, wo_v, sems,
               k_scr, vt_scr, wqt_scr, wot_scr, tmp_scr, pad_scr, tmpo_scr, pado_scr, wk_scr, wvt_scr, x_scr, q_scr, sa_scr, sb_scr, ot_scr, po_scr):
        i = pl.program_id(0)

        @pl.when(i == 0)
        def _():
            cp_w = [pltpu.make_async_copy(src, w_v.at[b], sems.at[b]) for b, src in enumerate((wa_hbm, wb_hbm))]
            cp_wo = [pltpu.make_async_copy(src, wo_v.at[b], sems.at[2 + b]) for b, src in enumerate((woa_hbm, wob_hbm))]
            cp_x = [pltpu.make_async_copy(xt_hbm.at[:, c * XW:(c + 1) * XW], xt_v.at[:, c * XW:(c + 1) * XW],
                                          sems.at[4 + c]) for c in range(XC)]
            cp_w[0].start()
            for c in range(XC):
                cp_x[c].start()
            cp_w[1].start()
            cp_wo[0].start()
            cp_wo[1].start()

            def prep_qkv(b):
                tmp_scr[b] = w_v[b].T.astype(F32)
                for part in (2, 1, 0):
                    for j in range(part * H, (part + 1) * H):
                        pad_scr[b, j * DP:j * DP + DH, :] = tmp_scr[b, j * DH:(j + 1) * DH, :]
                        pad_scr[b, j * DP + DH:(j + 1) * DP, :] = jnp.zeros((DP - DH, D), F32)
                    w = pad_scr[b, part * HP:(part + 1) * HP, :].astype(BF16)
                    if part == 2:
                        wvt_scr[b] = w
                    elif part == 1:
                        wk_scr[b] = w.T
                    else:
                        wqt_scr[b * HP:(b + 1) * HP, :] = w

            def prep_wo(b):
                tmpo_scr[b] = wo_v[b].astype(F32)
                for j in range(H):
                    pado_scr[b, j * DP:j * DP + DH, :] = tmpo_scr[b, j * DH:(j + 1) * DH, :]
                    pado_scr[b, j * DP + DH:(j + 1) * DP, :] = jnp.zeros((DP - DH, D), F32)
                wot_scr[:, b * HP:(b + 1) * HP] = pado_scr[b].astype(BF16).T

            def kv_chunk(b, c):
                vt = jnp.dot(wvt_scr[b], xt_v[:, c * XW:(c + 1) * XW], preferred_element_type=F32)
                row = jax.lax.broadcasted_iota(jnp.int32, vt.shape, 0)
                vt = jnp.where(row % DP == DH, 1.0, vt)
                vt_scr[b * H:(b + 1) * H, :, c * XW:(c + 1) * XW] = vt.astype(BF16).reshape(H, DP, XW)
                k = jnp.dot(x_scr[c * XW:(c + 1) * XW, :], wk_scr[b], preferred_element_type=F32)
                for g in range(G // 2):
                    k_scr[b * (G // 2) + g, c * XW:(c + 1) * XW, :] = k[:, g * 128:(g + 1) * 128].astype(BF16)

            cp_w[0].wait()
            prep_qkv(0)
            cp_x[0].wait()
            x_scr[0:XW, :] = xt_v[:, 0:XW].T
            kv_chunk(0, 0)
            for c in range(1, XC):
                cp_x[c].wait()
            cp_w[1].wait()
            cp_wo[0].wait()
            cp_wo[1].wait()
            for c in range(1, XC):
                x_scr[c * XW:(c + 1) * XW, :] = xt_v[:, c * XW:(c + 1) * XW].T
                if c == 1:
                    prep_qkv(1)
                if c == min(2, XC - 1):
                    prep_wo(0)
                    prep_wo(1)
                kv_chunk(0, c)
            for c in range(XC):
                kv_chunk(1, c)

        xq = xt_v[:, pl.ds(pl.multiple_of(i * TQ, TQ), TQ)]
        qt = jnp.dot(wqt_scr[...], xq, preferred_element_type=F32) * (DH ** -0.5 * LOG2E)
        q_scr[...] = qt.astype(BF16).reshape(G, 128, TQ)
        gl = jnp.dot(jnp.broadcast_to(gw_ref[...].reshape(1, D), (8, D)), xq, preferred_element_type=F32)
        gate = jax.nn.sigmoid(gl[0:1, :])

        rowg = jax.lax.broadcasted_iota(jnp.int32, (128, TQ), 0) // DP

        def stage(h1, s1_ref, h2, s2_ref, m2, extra=None):
            if h1 is not None:
                g = h1 // 4
                qg = q_scr[g]
                qm = jnp.where(rowg == (h1 % 4), qg, jnp.zeros_like(qg))
                mx = jnp.full((8, TQ), -jnp.inf, F32)
            if h2 is not None:
                acc = jnp.zeros((DP, TQ), F32)
            for cc in range(NC + LAG):
                if h1 is not None and cc < NC:
                    c = cc
                    s = jnp.dot(k_scr[g, c * KC:(c + 1) * KC, :], qm, preferred_element_type=F32)
                    s1_ref[c * KC:(c + 1) * KC, :] = s
                    mx = jnp.maximum(mx, s.reshape(KC // 8, 8, TQ).max(axis=0))
                if h2 is not None and cc >= LAG:
                    c = cc - LAG
                    p = jnp.exp2(s2_ref[c * KC:(c + 1) * KC, :] - m2).astype(BF16)
                    acc = acc + jnp.dot(vt_scr[h2, :, c * KC:(c + 1) * KC], p, preferred_element_type=F32)
                if extra is not None and cc < NC:
                    extra(cc)
            if h2 is not None:
                l = acc[DH:DH + 1, :]
                gsel = jnp.where(h2 < H, gate, 1.0 - gate)
                ot_scr[h2] = (acc * (gsel / l)).astype(BF16)
            if h1 is not None:
                return mx.max(axis=0, keepdims=True)
            return None

        bufs = (sa_scr, sb_scr)
        m = stage(0, sa_scr, None, None, None)
        NIT = (NH - 1) // U

        def body(j, m):
            for u in range(U):
                k = j * U + 1 + u
                m = stage(k, bufs[(1 + u) % 2], k - 1, bufs[u % 2], m)
            return m

        if NIT > 0:
            m = jax.lax.fori_loop(0, NIT, body, m)
        for k in range(NIT * U + 1, NH):
            m = stage(k, bufs[k % 2], k - 1, bufs[(k - 1) % 2], m)
        KS = (NH - 4) * DP
        RB = 64
        def extra(c):
            if c % 2 == 0 and c // 2 < D // RB:
                r = c // 2
                po_scr[r * RB:(r + 1) * RB, :] = jnp.dot(wot_scr[r * RB:(r + 1) * RB, :KS], ot_scr[:NH - 4].reshape(KS, TQ),
                                                         preferred_element_type=F32)
        stage(None, None, NH - 1, bufs[(NH - 1) % 2], m, extra)
        out = po_scr[...] + jnp.dot(wot_scr[:, KS:], ot_scr[NH - 4:].reshape(4 * DP, TQ), preferred_element_type=F32)
        o_ref[...] = out.astype(o_ref.dtype)

    def fn(A_x, A_wqkv, A_wo, B_x, B_wqkv, B_wo, gate_w):
        xt = jnp.transpose(A_x, (0, 2, 1)).reshape(D, S)
        gw = gate_w
        anyspec = pl.BlockSpec(memory_space=pl.ANY)
        out = pl.pallas_call(
            kernel,
            grid=(S // TQ,),
            in_specs=[anyspec, anyspec, anyspec, anyspec, anyspec, pl.BlockSpec((D,), lambda i: (0,))],
            out_specs=pl.BlockSpec((D, TQ), lambda i: (0, i)),
            out_shape=jax.ShapeDtypeStruct((D, S), BF16),
            scratch_shapes=[pltpu.VMEM((D, S), BF16),
                            pltpu.VMEM((2, D, 3 * D), BF16),
                            pltpu.VMEM((2, D, D), BF16),
                            pltpu.SemaphoreType.DMA((4 + XC,)),
                            pltpu.VMEM((G, S, 128), BF16),
                            pltpu.VMEM((NH, DP, S), BF16),
                            pltpu.VMEM((NH * DP, D), BF16),
                            pltpu.VMEM((D, NH * DP), BF16),
                            pltpu.VMEM((2, 3 * D, D), F32),
                            pltpu.VMEM((2, 3 * HP, D), F32),
                            pltpu.VMEM((2, D, D), F32),
                            pltpu.VMEM((2, HP, D), F32),
                            pltpu.VMEM((2, D, HP), BF16),
                            pltpu.VMEM((2, HP, D), BF16),
                            pltpu.VMEM((S, D), BF16),
                            pltpu.VMEM((G, 128, TQ), BF16),
                            pltpu.VMEM((S, TQ), F32),
                            pltpu.VMEM((S, TQ), F32),
                            pltpu.VMEM((NH, DP, TQ), BF16),
                            pltpu.VMEM((D, TQ), F32)],
            compiler_params=pltpu.CompilerParams(dimension_semantics=("arbitrary",), vmem_limit_bytes=100 * 2**20),
        )(xt, A_wqkv, B_wqkv, A_wo, B_wo, gw)
        return jnp.transpose(out.reshape(1, D, S), (0, 2, 1))
    return fn


_impl = make_kernel(512, 128, 6, 2, 2)


@jax.jit
def pallas_gated_mix__mha_block__softmax_full_mha__prompt_kernel(
    A_x: jax.Array,
    A_wqkv: jax.Array,
    A_wo: jax.Array,
    B_x: jax.Array,
    B_wqkv: jax.Array,
    B_wo: jax.Array,
    gate_w: jax.Array,
):
    return _impl(A_x, A_wqkv, A_wo, B_x, B_wqkv, B_wo, gate_w)
```

```python
import jax
import jax.numpy as jnp
from jax.experimental import pallas as pl
from jax.experimental.pallas import tpu as pltpu

S, D, H, DH = 2048, 448, 16, 28
DP = 32
HP = H * DP
NH = 2 * H
G = NH * DP // 128
LOG2E = 1.4426950408889634
F32, BF16 = jnp.float32, jnp.bfloat16

TQ = 512
KC = 128
U = 6
XC = 2
LAG = 2
NC = S // KC
XW = S // XC
RB = 64
KS = (NH - 4) * DP


def _kernel(xt_hbm, wa_hbm, wb_hbm, woa_hbm, wob_hbm, gw_ref, o_ref,
            xt_v, w_v, wo_v, sems,
            k_scr, vt_scr, wqt_scr, wot_scr, tmp_scr, pad_scr, tmpo_scr, pado_scr,
            wk_scr, wvt_scr, x_scr, q_scr, sa_scr, sb_scr, ot_scr, po_scr):
    i = pl.program_id(0)

    @pl.when(i == 0)
    def _():
        cp_w = [pltpu.make_async_copy(src, w_v.at[b], sems.at[b])
                for b, src in enumerate((wa_hbm, wb_hbm))]
        cp_wo = [pltpu.make_async_copy(src, wo_v.at[b], sems.at[2 + b])
                 for b, src in enumerate((woa_hbm, wob_hbm))]
        cp_x = [pltpu.make_async_copy(xt_hbm.at[:, c * XW:(c + 1) * XW],
                                      xt_v.at[:, c * XW:(c + 1) * XW], sems.at[4 + c])
                for c in range(XC)]
        cp_w[0].start()
        for c in range(XC):
            cp_x[c].start()
        cp_w[1].start()
        cp_wo[0].start()
        cp_wo[1].start()

        def prep_qkv(b):
            tmp_scr[b] = w_v[b].T.astype(F32)
            for part in (2, 1, 0):
                for j in range(part * H, (part + 1) * H):
                    pad_scr[b, j * DP:j * DP + DH, :] = tmp_scr[b, j * DH:(j + 1) * DH, :]
                    pad_scr[b, j * DP + DH:(j + 1) * DP, :] = jnp.zeros((DP - DH, D), F32)
                w = pad_scr[b, part * HP:(part + 1) * HP, :].astype(BF16)
                if part == 2:
                    wvt_scr[b] = w
                elif part == 1:
                    wk_scr[b] = w.T
                else:
                    wqt_scr[b * HP:(b + 1) * HP, :] = w

        def prep_wo(b):
            tmpo_scr[b] = wo_v[b].astype(F32)
            for j in range(H):
                pado_scr[b, j * DP:j * DP + DH, :] = tmpo_scr[b, j * DH:(j + 1) * DH, :]
                pado_scr[b, j * DP + DH:(j + 1) * DP, :] = jnp.zeros((DP - DH, D), F32)
            wot_scr[:, b * HP:(b + 1) * HP] = pado_scr[b].astype(BF16).T

        def kv_chunk(b, c):
            vt = jnp.dot(wvt_scr[b], xt_v[:, c * XW:(c + 1) * XW],
                         preferred_element_type=F32)
            row = jax.lax.broadcasted_iota(jnp.int32, vt.shape, 0)
            vt = jnp.where(row % DP == DH, 1.0, vt)
            vt_scr[b * H:(b + 1) * H, :, c * XW:(c + 1) * XW] = vt.astype(BF16).reshape(H, DP, XW)
            k = jnp.dot(x_scr[c * XW:(c + 1) * XW, :], wk_scr[b],
                        preferred_element_type=F32)
            for g in range(G // 2):
                k_scr[b * (G // 2) + g, c * XW:(c + 1) * XW, :] = (
                    k[:, g * 128:(g + 1) * 128].astype(BF16))

        cp_w[0].wait()
        prep_qkv(0)
        cp_x[0].wait()
        x_scr[0:XW, :] = xt_v[:, 0:XW].T
        kv_chunk(0, 0)
        for c in range(1, XC):
            cp_x[c].wait()
        cp_w[1].wait()
        cp_wo[0].wait()
        cp_wo[1].wait()
        for c in range(1, XC):
            x_scr[c * XW:(c + 1) * XW, :] = xt_v[:, c * XW:(c + 1) * XW].T
            if c == 1:
                prep_qkv(1)
                prep_wo(0)
                prep_wo(1)
            kv_chunk(0, c)
        for c in range(XC):
            kv_chunk(1, c)

    xq = xt_v[:, pl.ds(pl.multiple_of(i * TQ, TQ), TQ)]
    qt = jnp.dot(wqt_scr[...], xq, preferred_element_type=F32) * (DH ** -0.5 * LOG2E)
    q_scr[...] = qt.astype(BF16).reshape(G, 128, TQ)
    gl = jnp.dot(jnp.broadcast_to(gw_ref[...].reshape(1, D), (8, D)), xq,
                 preferred_element_type=F32)
    gate = jax.nn.sigmoid(gl[0:1, :])

    rowg = jax.lax.broadcasted_iota(jnp.int32, (128, TQ), 0) // DP

    def stage(h1, s1_ref, h2, s2_ref, m2, extra=None):
        if h1 is not None:
            g = h1 // 4
            qg = q_scr[g]
            qm = jnp.where(rowg == (h1 % 4), qg, jnp.zeros_like(qg))
            mx = jnp.full((8, TQ), -jnp.inf, F32)
        if h2 is not None:
            acc = jnp.zeros((DP, TQ), F32)
        for cc in range(NC + LAG):
            if h1 is not None and cc < NC:
                c = cc
                s = jnp.dot(k_scr[g, c * KC:(c + 1) * KC, :], qm,
                            preferred_element_type=F32)
                s1_ref[c * KC:(c + 1) * KC, :] = s
                mx = jnp.maximum(mx, s.reshape(KC // 8, 8, TQ).max(axis=0))
            if h2 is not None and cc >= LAG:
                c = cc - LAG
                p = jnp.exp2(s2_ref[c * KC:(c + 1) * KC, :] - m2).astype(BF16)
                acc = acc + jnp.dot(vt_scr[h2, :, c * KC:(c + 1) * KC], p,
                                    preferred_element_type=F32)
            if extra is not None and cc < NC:
                extra(cc)
        if h2 is not None:
            l = acc[DH:DH + 1, :]
            gsel = jnp.where(h2 < H, gate, 1.0 - gate)
            ot_scr[h2] = (acc * (gsel / l)).astype(BF16)
        if h1 is not None:
            return mx.max(axis=0, keepdims=True)
        return None

    bufs = (sa_scr, sb_scr)
    m = stage(0, sa_scr, None, None, None)
    nit = (NH - 1) // U

    def body(j, m):
        for u in range(U):
            k = j * U + 1 + u
            m = stage(k, bufs[(1 + u) % 2], k - 1, bufs[u % 2], m)
        return m

    m = jax.lax.fori_loop(0, nit, body, m)
    for k in range(nit * U + 1, NH):
        m = stage(k, bufs[k % 2], k - 1, bufs[(k - 1) % 2], m)

    def extra(c):
        if c % 2 == 0 and c // 2 < D // RB:
            r = c // 2
            po_scr[r * RB:(r + 1) * RB, :] = jnp.dot(
                wot_scr[r * RB:(r + 1) * RB, :KS], ot_scr[:NH - 4].reshape(KS, TQ),
                preferred_element_type=F32)

    stage(None, None, NH - 1, bufs[(NH - 1) % 2], m, extra)
    out = po_scr[...] + jnp.dot(wot_scr[:, KS:], ot_scr[NH - 4:].reshape(4 * DP, TQ),
                                preferred_element_type=F32)
    o_ref[...] = out.astype(o_ref.dtype)


@jax.jit
def pallas_gated_mix__mha_block__softmax_full_mha__prompt_kernel(
    A_x: jax.Array,
    A_wqkv: jax.Array,
    A_wo: jax.Array,
    B_x: jax.Array,
    B_wqkv: jax.Array,
    B_wo: jax.Array,
    gate_w: jax.Array,
):
    del B_x
    xt = jnp.transpose(A_x, (0, 2, 1)).reshape(D, S)
    anyspec = pl.BlockSpec(memory_space=pl.ANY)
    out = pl.pallas_call(
        _kernel,
        grid=(S // TQ,),
        in_specs=[anyspec, anyspec, anyspec, anyspec, anyspec,
                  pl.BlockSpec((D,), lambda i: (0,))],
        out_specs=pl.BlockSpec((D, TQ), lambda i: (0, i)),
        out_shape=jax.ShapeDtypeStruct((D, S), BF16),
        scratch_shapes=[
            pltpu.VMEM((D, S), BF16),
            pltpu.VMEM((2, D, 3 * D), BF16),
            pltpu.VMEM((2, D, D), BF16),
            pltpu.SemaphoreType.DMA((4 + XC,)),
            pltpu.VMEM((G, S, 128), BF16),
            pltpu.VMEM((NH, DP, S), BF16),
            pltpu.VMEM((NH * DP, D), BF16),
            pltpu.VMEM((D, NH * DP), BF16),
            pltpu.VMEM((2, 3 * D, D), F32),
            pltpu.VMEM((2, 3 * HP, D), F32),
            pltpu.VMEM((2, D, D), F32),
            pltpu.VMEM((2, HP, D), F32),
            pltpu.VMEM((2, D, HP), BF16),
            pltpu.VMEM((2, HP, D), BF16),
            pltpu.VMEM((S, D), BF16),
            pltpu.VMEM((G, 128, TQ), BF16),
            pltpu.VMEM((S, TQ), F32),
            pltpu.VMEM((S, TQ), F32),
            pltpu.VMEM((NH, DP, TQ), BF16),
            pltpu.VMEM((D, TQ), F32),
        ],
        compiler_params=pltpu.CompilerParams(
            dimension_semantics=("arbitrary",), vmem_limit_bytes=100 * 2**20),
    )(xt, A_wqkv, B_wqkv, A_wo, B_wo, gate_w)
    return jnp.transpose(out.reshape(1, D, S), (0, 2, 1))
```
